```python
import os as _os
_os.environ.setdefault("JAX_PLATFORMS", "cpu")
import jax
import jax.numpy as jnp

def _softmax(x, axis=-1):
    return jax.nn.softmax(x, axis=axis)
def _gelu(x):
    return jax.nn.gelu(x, approximate=True)
def _silu(x):
    return jax.nn.silu(x)
def _sigmoid(x):
    return jax.nn.sigmoid(x)
def _layernorm(x, axis=-1, eps=1e-5):
    m = jnp.mean(x, axis=axis, keepdims=True)
    v = jnp.var(x, axis=axis, keepdims=True)
    return (x - m) / jnp.sqrt(v + eps)
def _scatter_add(tgt, idx, src, axis=0):
    return tgt.at[idx].add(src)
def _segment_sum(src, seg, n):
    return jax.ops.segment_sum(src, seg, n)
class _Rng:
    def __init__(self, key):
        self._k = key
    def _next(self):
        self._k, sub = jax.random.split(self._k)
        return sub
    def normal(self, shape):
        return jax.random.normal(self._next(), shape, dtype=jnp.bfloat16)
    def randint(self, lo, hi, shape):
        return jax.random.randint(self._next(), shape, lo, hi, dtype=jnp.int32)
    def uniform(self, shape, lo=0.0, hi=1.0):
        return jax.random.uniform(self._next(), shape, jnp.bfloat16, lo, hi)
    def permutation(self, n):
        return jax.random.permutation(self._next(), n)


kernel_name = 'standalone__seq2seq_rnn_t_joint__speech'

def setup_inputs():
    _rng = _Rng(jax.random.key(int.from_bytes(__import__("os").urandom(4), "little")))
    _w = (lambda a: (lambda t: t.astype(jnp.bfloat16) if jnp.issubdtype(t.dtype, jnp.floating) else t)(jnp.asarray(a)))
    B, T, D, K = 2, 16000, 256, 31
    U = 8
    sc = (1.0 / (K * D)) ** 0.5
    sd = (1.0 / D) ** 0.5
    return {
        "x": _w((lambda *s: _rng.normal(s) * 0.2)(B, T, D) * 0.5),
        "w1": _w((lambda *s: _rng.normal(s) * 1.6)(K, D, D) * sc),
        "w2": _w((lambda *s: _rng.normal(s) * 1.6)(K, D, D) * sc),
        "g": _w((lambda *s: _rng.normal(s) * 1.6)(B, U, D) * 0.5),
        "w_f": _w((lambda *s: _rng.normal(s) * 1.6)(D, D) * sd),
        "w_g": _w((lambda *s: _rng.normal(s) * 1.6)(D, D) * sd),
        "w_o": _w((lambda *s: _rng.normal(s) * 1.6)(D, D) * sd),
    }

def reference(x, w1, w2, g, w_f, w_g, w_o):
    B, T, D = x.shape
    K = w1.shape[0]
    pad = K // 2
    xp = jnp.pad(x, ((0,0),(pad,pad),(0,0)))
    h = jnp.zeros_like(x)
    for i in range(K):
        h = h + jnp.einsum("btc,cd->btd", xp[:, i:i+T, :], w1[i])
    h = _gelu(h)[:, ::2, :]
    T1 = h.shape[1]
    hp = jnp.pad(h, ((0,0),(pad,pad),(0,0)))
    f = jnp.zeros_like(h)
    for i in range(K):
        f = f + jnp.einsum("btc,cd->btd", hp[:, i:i+T1, :], w2[i])
    f = _gelu(f)[:, ::2, :]
    fe = jnp.einsum("btd,de->bte", f, w_f)
    ge = jnp.einsum("bud,de->bue", g, w_g)
    j = jnp.tanh(fe[:, :, None, :] + ge[:, None, :, :])
    return jnp.einsum("btud,dv->btuv", j, w_o)
```

```python
import functools

import jax
import jax.numpy as jnp
import numpy as np
import jax.experimental.pallas as pl
import jax.experimental.pallas.tpu as pltpu

F32 = jnp.float32
BF16 = jnp.bfloat16
U32 = jnp.uint32


def _pre(d):
    if len(d) == 1:
        return d
    h = (len(d) + 1) // 4
    d0, d1, d2 = d[:2 * h - 1], d[h:3 * h - 1], d[2 * h:]
    return (_pre([a - b for a, b in zip(d0, d1)]) + _pre(d1)
            + _pre([a - b for a, b in zip(d2, d1)]))


def _wpre(w):
    if len(w) == 1:
        return w
    h = len(w) // 2
    return (_wpre(w[:h]) + _wpre([a + b for a, b in zip(w[:h], w[h:])])
            + _wpre(w[h:]))


def _post(get, lo, n):
    if n == 1:
        return [get(lo)]
    t = n // 3
    m0, m1, m2 = _post(get, lo, t), _post(get, lo + t, t), _post(get, lo + 2 * t, t)
    return [a + b for a, b in zip(m0, m1)] + [a + b for a, b in zip(m2, m1)]


_OUT_IN = {2: [(0, 1, -1), (1, 1, 0), (2, 1, -1)],
           3: [(0, 2, -1), (1, 2, 1), (2, 1, -1), (3, 1, -1)]}


def _outer_w(m, w0, w1):
    if m == 2:
        return [w0, w0 + w1, w1]
    return [w0, 0.5 * (w0 + w1), 0.5 * (w0 - w1), w1]


def _outer_out(m, y):
    if m == 2:
        return [y[0] + y[1], y[2] + y[1]]
    s = y[1] + y[2]
    return [y[0] + s, y[1] - y[2], y[3] + s]


def _gelu(x):
    c = float(np.sqrt(2.0 / np.pi))
    return 0.5 * x * (1.0 + jnp.tanh(c * (x + 0.044715 * (x * x * x))))


def _unpack(v, half):
    v = (v << 16) if half == 0 else (v & np.uint32(0xFFFF0000))
    return pltpu.bitcast(v, F32)


def _pack(lo, hi):
    return pltpu.bitcast(
        pltpu.pack_elementwise([lo, hi], packed_dtype=BF16), U32)


M1, M2 = 3, 2
Q1, Q2 = 336, 256
JT = 200


def _body(x_hbm, w1_hbm, w2_hbm, g_ref, wf_ref, wg_ref, wo_ref, o_hbm,
          w2raw, w1t, w2t, xa, xc, hb, lhs0, lhs1, y0, y1, p0, p1, fe, ob,
          sem, osem, *, T, U):
    T1, T2 = T // 2, T // 4
    XR = 8 * M1 * Q1 + 16
    HR = max(8 * M2 * Q2 + 16, 4 * M1 * Q1 + 8)
    FR = 8 * M2 * Q2

    def xcopies(b, dst):
        return [pltpu.make_async_copy(
            x_hbm.at[b, :, pl.ds(128 * l, 128)],
            dst.bitcast(BF16).at[l, pl.ds(16, T), :],
            sem.at[3 + 2 * b + l]) for l in range(2)]

    w1raw = lhs1.bitcast(BF16)
    wc = [pltpu.make_async_copy(w1_hbm.at[pl.ds(0, 16)],
                                w1raw.at[pl.ds(0, 16), pl.ds(0, 256), pl.ds(0, 256)],
                                sem.at[0]),
          pltpu.make_async_copy(w1_hbm.at[pl.ds(16, 15)],
                                w1raw.at[pl.ds(0, 15), pl.ds(0, 256), pl.ds(256, 256)],
                                sem.at[1]),
          pltpu.make_async_copy(w2_hbm, w2raw.bitcast(BF16), sem.at[2])]
    xa_c, xc_c = xcopies(0, xa), xcopies(1, xc)
    for c in wc + xa_c + xc_c:
        c.start()

    def zero(ref, lo, hi):
        ref[:, pl.ds(lo, hi - lo), :] = jnp.zeros((2, hi - lo, 128), U32)

    for r in (xa, xc):
        zero(r, 0, 8)
        zero(r, 8 + T1, XR)
    zero(hb, 0, 8)

    def al(i, n):
        return pl.ds(i * n if isinstance(i, int) else pl.multiple_of(i * n, n), n)

    def wtrans(raw, wt, m, half, r):
        ks = [2 * a - 1 + half for a in range(16)]
        u = [raw(k, al(r, 8)) if k >= 0 else None for k in ks]
        res = []
        for par in range(2):
            w = [jnp.zeros((8, 256), F32) if v is None else _unpack(v, par)
                 for v in u]
            outer = [_outer_w(m, w[c], w[8 + c]) for c in range(8)]
            res.append([v for gi in range(m + 1)
                        for v in _wpre([o[gi] for o in outer])])
        for n, (lo, hi) in enumerate(zip(*res)):
            wt[n, al(half * 16 + r, 8), :] = _pack(lo, hi)

    def preadd(src, m, gi, lhs, q, r, l):
        i, j, s = _OUT_IN[m][gi]
        P = 8 * m

        def ld(z, e):
            return src[l, pl.ds(r * (8 * P) + z * (q // 2) * P + e, 8, stride=P), :]
        for half in range(2):
            def val(e):
                v = _unpack(jnp.concatenate([ld(0, 8 * i + e), ld(1, 8 * i + e)]), half)
                if s:
                    u = _unpack(jnp.concatenate([ld(0, 8 * j + e), ld(1, 8 * j + e)]), half)
                    v = v + u if s > 0 else v - u
                return v

            def rec(d, n):
                if len(d) == 1:
                    lhs[n, al(r, 8), pl.ds(half * 256 + l * 128, 128)] = _pack(d[0][:8], d[0][8:])
                    return
                h = (len(d) + 1) // 4
                t = {4: 9, 2: 3, 1: 1}[h]
                d0, d1, d2 = d[:2 * h - 1], d[h:3 * h - 1], d[2 * h:]
                rec([u - v for u, v in zip(d0, d1)], n)
                e2 = [u - v for u, v in zip(d2, d1)]
                rec(d1, n + t)
                rec(e2, n + 2 * t)
            rec([val(e) for e in range(15)], 0)

    def put_h(dst, a):
        def f(v, t, z, l):
            q0 = t * 8 + z * (Q1 // 2)
            for r in range(0, 8, 2):
                dst[l, pl.ds(8 + q0 * (4 * M1) + 4 * a + r // 2, 8, stride=4 * M1), :] = (
                    _pack(_gelu(v[r]), _gelu(v[r + 1])))
        return f

    def put_f(b, a):
        def f(v, t, z, l):
            q0 = t * 8 + z * (Q2 // 2)
            for r in range(8):
                xc[l, pl.ds(b * FR + q0 * (8 * M2) + 8 * a + r, 8, stride=8 * M2), :] = (
                    pltpu.bitcast(_gelu(v[r]), U32))
        return f

    def keep(y):
        def f(v, t, z, l):
            for r in range(8):
                y[r, l, al(2 * t + z, 8), :] = v[r]
        return f

    def plus(y, then):
        def f(v, t, z, l):
            then([y[r, l, al(2 * t + z, 8), :] + v[r] for r in range(8)], t, z, l)
        return f

    def sumdiff(then):
        def f(v, t, z, l):
            p = [y0[r, l, al(2 * t + z, 8), :] for r in range(8)]
            keep(y1)([u + w for u, w in zip(p, v)], t, z, l)
            then([u - w for u, w in zip(p, v)], t, z, l)
        return f

    def post(p, q, then):
        def f(t):
            for z in range(2):
                for l in range(2):
                    m = [[p[k, r, l, pl.ds(t * 16 + z, 8, stride=2), :]
                          for r in range(4)] for k in range(3)]
                    then([u + w for u, w in zip(m[0], m[1])]
                         + [u + w for u, w in zip(m[2], m[1])], t, z, l)
        return f, q // 16

    def pre(src, m, gi, lhs, q):
        def f(r):
            for l in range(2):
                preadd(src, m, gi, lhs, q, r, l)
        return f, q // 16

    def stage(tag, lhs, p, wt, gi, q, *tasks):
        def run(k, c):
            def get(n):
                kk = k * 9 + n
                for f, nt in tasks:
                    for i in range(nt * kk // 27, nt * (kk + 1) // 27):
                        f(i)
                return jnp.dot(
                    pltpu.bitcast(lhs[k * 9 + n, pl.ds(0, q // 2), :], BF16),
                    pltpu.bitcast(wt[gi * 27 + k * 9 + n], BF16),
                    preferred_element_type=F32)
            for r, v in enumerate(_post(get, 0, 9)):
                for l in range(2):
                    p[k, r, l, pl.ds(0, q), :] = v[:, 128 * l:128 * l + 128]
            return c
        with jax.named_scope(tag):
            for k in range(3):
                run(k, 0)

    wc[0].wait()
    wc[1].wait()
    for half in range(2):
        def f(r, c):
            wtrans(lambda k, rs: lhs1[k % 16, rs, pl.ds(256 * (k // 16), 256)],
                   w1t, M1, half, r)
            return c
        jax.lax.fori_loop(0, 16, f, 0)
    wc[2].wait()
    for half in range(2):
        def f(r, c):
            wtrans(lambda k, rs: w2raw[k, rs, :], w2t, M2, half, r)
            return c
        jax.lax.fori_loop(0, 16, f, 0)
    for l in range(2):
        xa_c[l].wait()

        def f(r, c):
            preadd(xa, M1, 1, lhs0, Q1, r, l)
            return c
        jax.lax.fori_loop(0, Q1 // 16, f, 0)

    ev, od = (lhs0, p0), (lhs1, p1)
    stage("A1", *ev, w1t, 1, Q1, pre(xa, M1, 2, lhs1, Q1))
    stage("A2", *od, w1t, 2, Q1, pre(xa, M1, 0, lhs0, Q1), post(p0, Q1, keep(y0)))
    stage("A0", *ev, w1t, 0, Q1, pre(xa, M1, 3, lhs1, Q1), post(p1, Q1, sumdiff(put_h(hb, 1))))
    for c in xc_c:
        c.wait()
    stage("A3", *od, w1t, 3, Q1, pre(xc, M1, 1, lhs0, Q1), post(p0, Q1, plus(y1, put_h(hb, 0))))
    stage("B1", *ev, w1t, 1, Q1, pre(xc, M1, 2, lhs1, Q1), post(p1, Q1, plus(y1, put_h(hb, 2))))
    zero(hb, 8 + T1 // 2, HR)
    stage("B2", *od, w1t, 2, Q1, pre(xc, M1, 0, lhs0, Q1), post(p0, Q1, keep(y0)))
    stage("B0", *ev, w1t, 0, Q1, pre(xc, M1, 3, lhs1, Q1), post(p1, Q1, sumdiff(put_h(xa, 1))))
    stage("B3", *od, w1t, 3, Q1, pre(hb, M2, 1, lhs0, Q2), post(p0, Q1, plus(y1, put_h(xa, 0))))
    stage("a1", *ev, w2t, 1, Q2, pre(hb, M2, 0, lhs1, Q2), post(p1, Q1, plus(y1, put_h(xa, 2))))
    zero(xa, 8 + T1 // 2, HR)
    stage("a0", *od, w2t, 0, Q2, pre(hb, M2, 2, lhs0, Q2), post(p0, Q2, keep(y0)))
    stage("a2", *ev, w2t, 2, Q2, pre(xa, M2, 1, lhs1, Q2), post(p1, Q2, plus(y0, put_f(0, 0))))
    stage("b1", *od, w2t, 1, Q2, pre(xa, M2, 0, lhs0, Q2), post(p0, Q2, plus(y0, put_f(0, 1))))
    stage("b0", *ev, w2t, 0, Q2, pre(xa, M2, 2, lhs1, Q2), post(p1, Q2, keep(y0)))
    stage("b2", *od, w2t, 2, Q2, post(p0, Q2, plus(y0, put_f(1, 0))))
    last, n_last = post(p1, Q2, plus(y0, put_f(1, 1)))

    def ocopy(b, c, slot):
        return pltpu.make_async_copy(
            ob.at[slot], o_hbm.at[b, pl.ds(c * (JT * U), JT * U), :], osem.at[slot])

    NC = T2 // JT

    for b in range(2):
        ge = jnp.dot(g_ref[b], wg_ref[...], preferred_element_type=F32)

        def chunk(c, carry):
            slot = c % 2

            @pl.when(c >= 2)
            def _():
                ocopy(b, c - 2, slot).wait()

            ts = pl.ds(pl.multiple_of(b * FR + c * JT, 8), JT)
            f = pltpu.bitcast(
                jnp.concatenate([xc[0, ts, :], xc[1, ts, :]], axis=1), F32)
            fe[...] = jnp.dot(f.astype(BF16), wf_ref[...],
                              preferred_element_type=F32)
            j = jnp.concatenate(
                [jnp.tanh(jnp.broadcast_to(fe[pl.ds(t, 1), :], (U, 256)) + ge)
                 for t in range(JT)], axis=0).astype(BF16)
            o = jnp.dot(j, wo_ref[...], preferred_element_type=F32)
            if b == 0:
                last(jnp.minimum(c, n_last - 1))
            ob[slot] = o.astype(ob.dtype)
            ocopy(b, c, slot).start()
            return carry
        with jax.named_scope("joint"):
            jax.lax.fori_loop(0, NC, chunk, 0)
        ocopy(b, NC - 2, (NC - 2) % 2).wait()
        ocopy(b, NC - 1, (NC - 1) % 2).wait()


@jax.jit
def pallas_standalone__seq2seq_rnn_t_joint__speech_kernel(
    x: jax.Array,
    w1: jax.Array,
    w2: jax.Array,
    g: jax.Array,
    w_f: jax.Array,
    w_g: jax.Array,
    w_o: jax.Array,
):
    B, T, D = x.shape
    K = w1.shape[0]
    U = g.shape[1]
    assert (B, T, D, K, U) == (2, 16000, 256, 31, 8) and x.dtype == BF16
    hbm = pl.BlockSpec(memory_space=pl.ANY)
    vmem = pl.BlockSpec(memory_space=pltpu.VMEM)
    out = pl.pallas_call(
        functools.partial(_body, T=T, U=U),
        in_specs=[hbm, hbm, hbm, vmem, vmem, vmem, vmem],
        out_specs=hbm,
        out_shape=jax.ShapeDtypeStruct((B, T // 4 * U, D), x.dtype),
        scratch_shapes=[
            pltpu.VMEM((K, D // 2, D), U32),
            pltpu.VMEM((27 * (M1 + 1), D, D), U32),
            pltpu.VMEM((27 * (M2 + 1), D, D), U32),
            pltpu.VMEM((2, 8 * M1 * Q1 + 16, 128), U32),
            pltpu.VMEM((2, max(8 * M1 * Q1 + 16, 16 * M2 * Q2), 128), U32),
            pltpu.VMEM((2, max(8 * M2 * Q2 + 16, 4 * M1 * Q1 + 8), 128), U32),
            *[pltpu.VMEM((27, Q1 // 2, 2 * D), U32)] * 2,
            *[pltpu.VMEM((8, 2, Q1, 128), F32)] * 2,
            *[pltpu.VMEM((3, 4, 2, Q1, 128), F32)] * 2,
            pltpu.VMEM((JT, D), F32),
            pltpu.VMEM((2, JT * U, D), x.dtype),
            pltpu.SemaphoreType.DMA((7,)),
            pltpu.SemaphoreType.DMA((2,)),
        ],
        compiler_params=pltpu.CompilerParams(vmem_limit_bytes=124 << 20),
    )(x, w1, w2, g, w_f, w_g, w_o)
    return out.reshape(B, T // 4, U, D)
```

```python
import functools

import jax
import jax.numpy as jnp
import numpy as np
import jax.experimental.pallas as pl
import jax.experimental.pallas.tpu as pltpu

F32 = jnp.float32
BF16 = jnp.bfloat16
U32 = jnp.uint32


_OUTER = ((0, 2, -1), (1, 2, 1), (2, 1, -1), (3, 1, -1))

QA, QB = 88, 80
XQ = QA + QB + 8
HQ = 384
KT = 2 * QA
NP = 7
NC = (QA + QB) // 8


def _wpre(w):
    w = w[None]
    for h in (4, 2, 1):
        lo, hi = w[:, :h], w[:, h:]
        w = jnp.stack([lo, lo + hi, hi], axis=1).reshape(-1, h, *w.shape[2:])
    return w[:, 0]


def _pre(d, h):
    d1 = d[:, h:3 * h - 1]
    return [d[:, :2 * h - 1] - d1, d1, d[:, 2 * h:] - d1]


def _post(v, gated):
    for g, h in ((9, 1), (3, 2), (1, 4)):
        v = v.reshape(g, 3, h, 8, 128)
        m = gated(v[:, 1]) if h == 1 else v[:, 1]
        v = jnp.concatenate([v[:, 0] + m, v[:, 2] + m], axis=1)
    return v[0]


def _runs(e0, n, period):
    k = min(n, period - e0 % period)
    return [(0, k)] + ([(k, n - k)] if k < n else [])


def _gelu2(x):
    c = float(np.sqrt(2.0 / np.pi))
    return x + x * jnp.tanh(x * (c + (c * 0.044715) * (x * x)))


def _unpack(v, half):
    v = (v << 16) if half == 0 else (v & np.uint32(0xFFFF0000))
    return pltpu.bitcast(v, F32)


def _pack(lo, hi):
    return pltpu.bitcast(
        pltpu.pack_elementwise([lo, hi], packed_dtype=BF16), U32)


def _body(x_hbm, w1_hbm, w2_hbm, g_ref, wf_ref, wg_ref, wo_ref, o_hbm,
          w1t, w2t, xp, hp, b0, b1, b2, y0, y1, fe0, fe1, wf2, ob, zr, zs, sem, osem, *, T):

    def rows(i, n=8):
        return pl.ds(i if isinstance(i, int) else pl.multiple_of(i, 8), n)

    def zero(ref, s0, ns, lo, n):
        ref[pl.ds(s0, ns), pl.ds(lo, n), :] = jnp.zeros((ns, n, 128), U32)

    def wcopies(w_hbm, wt, s):
        return [pltpu.make_async_copy(
            w_hbm.at[k], wt.bitcast(BF16).at[
                81 + (k + 1) // 2, pl.ds(256 * ((k + 1) % 2), 256), :],
            sem.at[s]) for k in range(31)]

    def staged(first, p, t):
        if first:
            return (b1, b2)[p // 2], (p % 2) * (QA // 8 + 1) + t
        return hp, p * (QB // 8) + t - QA // 8

    def xcopies(first, t, s):
        lo, hi = max(384 * t - 8, 0), min(384 * t + 376, T // 2)
        if first and t == QA // 8:
            hi = lo + 16
        off, res = lo - (384 * t - 8), []
        for p in range(4):
            ref, slot = staged(first, p, t)
            if off:
                zero(ref, slot, 1, 0, off)
            if off + hi - lo < 384:
                zero(ref, slot, 1, off + hi - lo, 384 - (off + hi - lo))
            res.append(pltpu.make_async_copy(
                x_hbm.at[p // 2, pl.ds(2 * lo, 2 * (hi - lo)),
                         pl.ds(128 * (p % 2), 128)],
                ref.bitcast(BF16).at[slot, pl.ds(2 * off, 2 * (hi - lo)), :],
                sem.at[s]))
        return res

    seen, tick = {}, [None]

    def gated(v):
        if tick[0] is None:
            return v
        return pltpu.bitcast(pltpu.bitcast(v, U32) | tick[0], v.dtype)

    def unpack(v, half):
        if tick[0] is None:
            return _unpack(v, half)
        c = tick[0] | np.uint32(0xFFFF0000 if half else 16)
        return pltpu.bitcast((v & c) if half else (v << c), F32)

    def wtrans(wt, scale, gi, half, l, r):
        rs, cs = rows(half * 128 + r * 8), pl.ds(128 * l, 128)
        if gi != 3:
            lo = wt[pl.ds(82 - half, 7 + half), rs, cs]
            if not half:
                lo = jnp.concatenate([jnp.zeros((1, 8, 128), U32), lo])
        if gi != 0:
            hi = wt[pl.ds(89, 8), rs, cs]
        res = []
        for par in range(2):
            if gi == 0:
                w = unpack(lo, par)
            elif gi == 3:
                w = unpack(hi, par)
            elif gi == 1:
                w = unpack(lo, par) + unpack(hi, par)
            else:
                w = unpack(lo, par) - unpack(hi, par)
            k = scale * (0.5 if gi in (1, 2) else 1.0)
            res.append(_wpre(w if k == 1.0 else k * w))
        wt[pl.ds(27 * gi, 27), rs, cs] = _pack(*res)
        seen[4] = lambda z: wt[27 * gi, rows(half * 128 + r * 8 + z), cs]

    def wtasks(wt, scale, *gis):
        return [functools.partial(wtrans, wt, scale, gi, half, l, r) for gi in gis
                for half in range(2) for l in range(2) for r in range(16)]

    def deint(first, p, t, e0):
        ref, slot = staged(first, p, t)
        xp[pl.ds(48 * p + e0, 24), rows(8 * t), :] = gated(jnp.stack(
            [ref[slot, pl.ds(e0 + e, 8, stride=48), :] for e in range(24)]))
        seen[2] = lambda z: xp[48 * p + e0, rows(8 * t + z), :]

    def preadd(ld, gi, dst, r, l, half):
        i, j, s = _OUTER[gi]
        u, v = unpack(ld(8 * i), half), unpack(ld(8 * j), half)
        o = (2 * half + l) * KT + r * 8
        for k, d in enumerate(_pre((u + v if s > 0 else u - v)[None], 4)):
            d = jnp.concatenate(_pre(d, 2))
            d = jnp.concatenate(_pre(d, 1), axis=1).reshape(9, 2, 8, 128)
            dst[pl.ds(1 + 9 * k, 9), rows(o), :] = _pack(d[:, 0], d[:, 1])
        seen[5] = lambda z: dst[27, rows(o + z), :]

    def pre1(q0, nq, gi, dst):
        def f(c, l, t, half):
            def ld(e):
                e += 24 * c
                return jnp.stack([jnp.concatenate([
                    xp[pl.ds((2 * b + l) * 48 + (e + k) % 48, n),
                       pl.ds(q0 + t * 8 + (e + k) // 48, 8), :]
                    for k, n in _runs(e, 15, 48)]) for b in range(2)], axis=1)
            preadd(ld, gi, dst, c * (nq // 8) + t, l, half)
        return [functools.partial(f, c, l, t, half) for t in range(nq // 8)
                for c in range(2) for l in range(2) for half in range(2)]

    def pre2(gi, dst):
        def f(r, l, half):
            def ld(e):
                return jnp.concatenate([
                    hp[pl.ds(l * 24 + (e + k) % 24, n),
                       pl.ds(16 * r + 2 * ((e + k) // 24), 16), :]
                    for k, n in _runs(e, 15, 24)]).reshape(15, 2, 8, 128)
            preadd(ld, gi, dst, r, l, half)
        return [functools.partial(f, r, l, half)
                for r in range(NC) for l in range(2) for half in range(2)]

    def act(v):
        v = _gelu2(v).reshape(4, 2, 8, 128)
        return _pack(v[:, 0], v[:, 1])

    def put_h(q0, nq, a):
        def f(v, t, l):
            c, tt = divmod(t, nq // 4)
            e = 12 * c + 4 * a + 8
            s, o = l * 24 + e % 24, 2 * q0 + 8 * tt + 2 * (e // 24)
            hp[pl.ds(s, 4), pl.ds(o, 8), :] = act(v)
            seen[1] = lambda z: hp[s, pl.ds(o + z, 8), :]
        return f

    def put_f(a):
        def f(v, t, l):
            s, o = (t // 22) * 24 + l * 12 + 4 * a, 8 * (t % 22)
            xp[pl.ds(s, 4), rows(o), :] = act(v)
            seen[2] = lambda z: xp[s, rows(o + z), :]
        return f

    def ys(t, l):
        return pl.ds(8 * l, 8), rows(8 * t), slice(None)

    def keep(y):
        def f(v, t, l):
            y[ys(t, l)] = v
            seen[3] = lambda z: pltpu.bitcast(y[8 * l, rows(8 * t + z), :], U32)
        return f

    def plus(then):
        def f(v, t, l):
            then(y1[ys(t, l)] + v, t, l)
        return f

    def sumdiff(then):
        def f(v, t, l):
            p = y0[ys(t, l)]
            keep(y1)(p + v, t, l)
            then(p - v, t, l)
        return f

    def post1(src, then, t, l):
        v = src[pl.ds(0, 27), rows(l * 2 * KT + 8 * t), :]
        then(_post(pltpu.bitcast(v, F32), gated), t, l)

    def post(src, nq, then):
        return [functools.partial(post1, src, then, t, l)
                for t in range(nq // 2) for l in range(2)]

    def stage(tag, buf, wt, gi, nq, *tasks):
        z = zs[0]

        @pl.when(z == 0)
        @jax.named_scope(tag)
        def run():
            nt, ns = nq // 2, 27 * (2 * NP - 1)
            gates = [None, None]
            ts = [f for _, _, f in sorted(
                ((i + 0.5) / len(x), j, f)
                for j, x in enumerate(tasks) for i, f in enumerate(x))]
            seen.clear()
            for n in range(27):
                k0 = 2 if gi == 0 and n == 0 else 0
                wn = wt[gi * 27 + n, pl.ds(64 * k0, 256 - 64 * k0), :]
                gate = gates.pop(0)
                if gate is not None:
                    wn = wn | jnp.tile(gate & zr[...], (32, 2))
                a = jnp.concatenate(
                    [buf[n + 1, pl.ds(k * KT, 2 * nq), :]
                     for k in range(k0, 4)], axis=1)
                v = pltpu.bitcast(
                    jnp.dot(pltpu.bitcast(a, BF16),
                            pltpu.bitcast(wn, BF16),
                            preferred_element_type=F32), U32)
                for l in range(2):
                    for p in range(NP):
                        lo, hi = 8 * (nt * p // NP), 8 * (nt * (p + 1) // NP)
                        w = v[lo:hi, 128 * l:128 * l + 128]
                        buf[n, pl.ds(l * 2 * KT + lo, hi - lo), :] = w
                        tick[0] = buf[n, rows(l * 2 * KT + lo + z), :] & zr[...]
                        k = l * NP + p
                        if k == 2 * NP - 1:
                            gates.append(functools.reduce(
                                jnp.bitwise_or, [f(z) for f in seen.values()],
                                tick[0]))
                            seen.clear()
                            continue
                        k += n * (2 * NP - 1)
                        for f in ts[len(ts) * k // ns:len(ts) * (k + 1) // ns]:
                            f()
            tick[0] = None

    def loop(n, f):
        def g(i, c):
            f(i)
            return c
        jax.lax.fori_loop(0, n, g, 0)

    xac = [xcopies(True, t, 3 + t) for t in range(QA // 8 + 1)]
    w1c, w2c = wcopies(w1_hbm, w1t, 0), wcopies(w2_hbm, w2t, 1)
    for c in w1c:
        c.start()
    xbc = [c for t in range(QA // 8, NC) for c in xcopies(False, t, 2)]
    zero(xp, 0, 192, QA + QB, 8)
    zs[0] = 0
    zr[...] = jnp.zeros((8, 128), U32)
    wf2[...] = (0.5 * wf_ref[...].astype(F32)).astype(BF16)

    A, B, Q = (0, QA), (QA, QB), (QA + QB) // 2
    for c in xac[0]:
        c.start()
    with jax.named_scope("wwait"):
        for c in w1c:
            c.wait()
    for cs in xac[1:]:
        for c in cs:
            c.start()
    with jax.named_scope("wt"):
        def wall(half, l, r):
            for gi in (1, 2, 0, 3):
                wtrans(w1t, 1.0, gi, half, l, r)
        for half in range(2):
            for l in range(2):
                loop(16, functools.partial(wall, half, l))
    with jax.named_scope("prologue"):
        first = pre1(*A, 1, b0)
        for t, cs in enumerate(xac):
            for c in cs:
                c.wait()
            if t == len(xac) - 2:
                for c in xbc + w2c:
                    c.start()
            for p in range(4):
                for e0 in (0, 24):
                    deint(True, p, t, e0)
            for f in first[8 * max(t - 1, 0):8 * t]:
                f()

    db = [functools.partial(deint, False, p, t, e0)
          for t in range(QA // 8, NC) for p in range(4) for e0 in (0, 24)]
    stage("A1", b0, w1t, 1, QA, pre1(*A, 2, b1))
    for c in xbc:
        c.wait()
    stage("A2", b1, w1t, 2, QA, pre1(*A, 0, b2), post(b0, QA, keep(y0)), db)
    for c in w2c:
        c.wait()
    for l in range(2):
        zero(hp, 24 * l, 8, 0, 8)
    stage("A0", b2, w1t, 0, QA, pre1(*A, 3, b0), post(b1, QA, sumdiff(put_h(*A, 1))))
    stage("A3", b0, w1t, 3, QA, pre1(*B, 1, b1), post(b2, QA, plus(put_h(*A, 0))))
    stage("B1", b1, w1t, 1, QB, pre1(*B, 2, b2), post(b0, QA, plus(put_h(*A, 2))))
    stage("B2", b2, w1t, 2, QB, pre1(*B, 0, b0), post(b1, QB, keep(y0)),
          wtasks(w2t, 0.5, 1))
    stage("B0", b0, w1t, 0, QB, pre1(*B, 3, b1), post(b2, QB, sumdiff(put_h(*B, 1))))
    c1 = pre2(1, b2)
    early = 4 * ((2 * QA - 2) // 16)
    stage("B3", b1, w1t, 3, QB, c1[:early], post(b0, QB, plus(put_h(*B, 0))),
          wtasks(w2t, 0.5, 2))
    with jax.named_scope("gap"):
        for f in post(b1, QB, plus(put_h(*B, 2))):
            f()
        end = 2 * ((T // 4 + 8) // 24)
        zero(hp, 0, 48, end, 8)
        for f in c1[early:]:
            f()
    stage("C1", b2, w2t, 1, Q, pre2(2, b0), wtasks(w2t, 0.5, 0, 3))
    stage("C2", b0, w2t, 2, Q, pre2(0, b1), post(b2, Q, keep(y0)))
    stage("C0", b1, w2t, 0, Q, pre2(3, b2), post(b0, Q, sumdiff(put_f(1))))
    stage("C3", b2, w2t, 3, Q, post(b1, Q, plus(put_f(0))))

    def last(c):
        for k in range(2):
            for l in range(2):
                post1(b2, plus(put_f(2)), 2 * c + k, l)

    def ocopy(c, slot, b, n=1536):
        return pltpu.make_async_copy(
            ob.at[slot, b, pl.ds(0, n), :],
            o_hbm.at[b, pl.ds(c * 1536, n), :], osem.at[slot, b])

    ge = [jnp.dot(g_ref[b], wg_ref[...], preferred_element_type=F32)
          for b in range(2)]

    def enc(c, fe):
        f = jnp.concatenate([
            xp[pl.ds((c // 11) * 24 + l * 12, 12), rows(16 * (c % 11), 16), :
               ].reshape(192, 128) for l in range(2)], axis=1)
        fe[...] = jnp.dot(pltpu.bitcast(f, BF16), wf2[...],
                          preferred_element_type=F32)

    def joint(fe, slot, nt):
        j = []
        for b in range(2):
            for t in range(nt):
                q, ph = divmod(t, 24)
                row = 32 * (ph // 2) + 2 * (2 * (2 * (q % 4) + b) + q // 4) + ph % 2
                j.append(jnp.broadcast_to(fe[pl.ds(row, 1), :], (8, 256)) + ge[b])
        o = jnp.dot(jnp.tanh(jnp.concatenate(j)).astype(BF16), wo_ref[...],
                    preferred_element_type=F32).astype(ob.dtype)
        for b in range(2):
            ob[slot, b, pl.ds(0, 8 * nt), :] = o[8 * nt * b:8 * nt * (b + 1)]

    def chunk(c, slot, wait=True, more=True):
        cur, nxt = (fe0, fe1) if slot == 0 else (fe1, fe0)
        enc(c + 1, nxt)
        if more:
            last(c + 2)
        if wait:
            for b in range(2):
                ocopy(c - 2, slot, b).wait()
        joint(cur, slot, 192)
        for b in range(2):
            ocopy(c, slot, b).start()

    with jax.named_scope("joint"):
        last(0)
        enc(0, fe0)
        last(1)
        chunk(0, 0, wait=False)
        chunk(1, 1, wait=False)

        def group(i):
            for k in range(4):
                chunk(2 + 4 * i + k, k % 2)
        loop(4, group)
        chunk(NC - 3, 0)
        chunk(NC - 2, 1, more=False)
        c = NC - 1
        nt = T // 4 - 192 * c
        for b in range(2):
            ocopy(c - 2, 0, b).wait()
        joint(fe0, 0, nt)
        for b in range(2):
            ocopy(c, 0, b, 8 * nt).start()
        for b in range(2):
            ocopy(c - 1, 1, b).wait()
            ocopy(c, 0, b, 8 * nt).wait()


@jax.jit
def pallas_standalone__seq2seq_rnn_t_joint__speech_kernel(
    x: jax.Array,
    w1: jax.Array,
    w2: jax.Array,
    g: jax.Array,
    w_f: jax.Array,
    w_g: jax.Array,
    w_o: jax.Array,
):
    B, T, D = x.shape
    K = w1.shape[0]
    U = g.shape[1]
    assert (B, T, D, K, U) == (2, 16000, 256, 31, 8) and x.dtype == BF16
    hbm = pl.BlockSpec(memory_space=pl.ANY)
    vmem = pl.BlockSpec(memory_space=pltpu.VMEM)
    out = pl.pallas_call(
        functools.partial(_body, T=T),
        in_specs=[hbm, hbm, hbm, vmem, vmem, vmem, vmem],
        out_specs=hbm,
        out_shape=jax.ShapeDtypeStruct((B, T // 4 * U, D), x.dtype),
        scratch_shapes=[
            *[pltpu.VMEM((108, D, D), U32)] * 2,
            pltpu.VMEM((192, XQ, 128), U32),
            pltpu.VMEM((48, HQ, 128), U32),
            *[pltpu.VMEM((28, 4 * KT, 128), U32)] * 3,
            *[pltpu.VMEM((16, 2 * KT, 128), F32)] * 2,
            *[pltpu.VMEM((384, D), F32)] * 2,
            pltpu.VMEM((D, D), BF16),
            pltpu.VMEM((2, 2, 1536, D), x.dtype),
            pltpu.VMEM((8, 128), U32),
            pltpu.SMEM((1,), jnp.int32),
            pltpu.SemaphoreType.DMA((15,)),
            pltpu.SemaphoreType.DMA((2, 2)),
        ],
        compiler_params=pltpu.CompilerParams(vmem_limit_bytes=126 << 20),
    )(x, w1, w2, g, w_f, w_g, w_o)
    return out.reshape(B, T // 4, U, D)
```
